```python
import jax
import jax.numpy as jnp

def _softmax(x, axis=-1):
    return jax.nn.softmax(x, axis=axis)

def _gelu(x):
    return jax.nn.gelu(x, approximate=True)

def _silu(x):
    return jax.nn.silu(x)

def _sigmoid(x):
    return jax.nn.sigmoid(x)

def _layernorm(x, axis=-1, eps=1e-05):
    m = jnp.mean(x, axis=axis, keepdims=True)
    v = jnp.var(x, axis=axis, keepdims=True)
    return (x - m) / jnp.sqrt(v + eps)

def _scatter_add(tgt, idx, src, axis=0):
    return tgt.at[idx].add(src)

def _segment_sum(src, seg, n):
    return jax.ops.segment_sum(src, seg, n)

class _Rng:

    def __init__(self, key):
        self._k = key

    def _next(self):
        self._k, sub = jax.random.split(self._k)
        return sub

    def normal(self, shape):
        return jax.random.normal(self._next(), shape, dtype=jnp.bfloat16)

    def randint(self, lo, hi, shape):
        return jax.random.randint(self._next(), shape, lo, hi, dtype=jnp.int32)

    def uniform(self, shape, lo=0.0, hi=1.0):
        return jax.random.uniform(self._next(), shape, jnp.bfloat16, lo, hi)

    def permutation(self, n):
        return jax.random.permutation(self._next(), n)
kernel_name = 'interleave_layers__linear_kernel_hedgehog__mixer_gmlp__prompt'

def _fwd_setup_inputs():
    _rng = _Rng(jax.random.key(int.from_bytes(__import__("os").urandom(4), "little")))
    _w = lambda a: (lambda t: t.astype(jnp.bfloat16) if jnp.issubdtype(t.dtype, jnp.floating) else t)(jnp.asarray(a))

    def _A_setup():
        B, S, D, H = (1, 2048, 640, 32)
        Dh = D // H
        return {'x': _w((lambda *s: _rng.normal(s) * 0.05)(B, S, D)), 'wqkv': _w((lambda *s: _rng.normal(s) * 0.05)(D, 3 * D)), 'w_phi': _w((lambda *s: _rng.normal(s) * 0.05)(H, Dh, Dh) * Dh ** (-0.5)), 'wo': _w((lambda *s: _rng.normal(s) * 0.05)(D, D))}
    _A_in = _A_setup()

    def _B_setup():
        B, S, D, F = (1, 2048, 640, 1536)
        Fh = F // 2
        return {'x': _w((lambda *s: _rng.normal(s) * 0.05)(B, S, D)), 'w_in': _w((lambda *s: _rng.normal(s) * 0.05)(D, 2 * Fh)), 'w_sp': _w(0.01 * (lambda *s: _rng.normal(s) * 0.05)(S, S)), 'b_sp': _w(1.0 + 0.01 * (lambda *s: _rng.normal(s) * 0.05)(S)), 'w_out': _w((lambda *s: _rng.normal(s) * 0.05)(Fh, D))}
    _B_in = _B_setup()
    return {'A_x': _A_in['x'], 'A_wqkv': _A_in['wqkv'], 'A_w_phi': _A_in['w_phi'], 'A_wo': _A_in['wo'], 'B_x': _B_in['x'], 'B_w_in': _B_in['w_in'], 'B_w_sp': _B_in['w_sp'], 'B_b_sp': _B_in['b_sp'], 'B_w_out': _B_in['w_out']}

def _fwd_reference(A_x, A_wqkv, A_w_phi, A_wo, B_x, B_w_in, B_w_sp, B_b_sp, B_w_out):

    def _A_ref(x, wqkv, w_phi, wo):
        B, S, D = x.shape
        H = 32
        Dh = D // H
        qkv = (lambda x, *d: x.transpose(*d))((x @ wqkv).reshape(B, S, 3, H, Dh), 2, 0, 3, 1, 4)
        q, k, v = (qkv[0], qkv[1], qkv[2])
        pq = jnp.einsum('bhsd,hdf->bhsf', q, w_phi)
        pk = jnp.einsum('bhsd,hdf->bhsf', k, w_phi)
        phi_q = jnp.concatenate([_softmax(pq, axis=-1), _softmax(-pq, axis=-1)], axis=-1)
        phi_k = jnp.concatenate([_softmax(pk, axis=-1), _softmax(-pk, axis=-1)], axis=-1)
        kv = jnp.einsum('bhsf,bhsd->bhfd', phi_k, v)
        z = jnp.einsum('bhsf->bhf', phi_k)
        num = jnp.einsum('bhqf,bhfd->bhqd', phi_q, kv)
        den = jnp.einsum('bhqf,bhf->bhq', phi_q, z)[..., None] + 1e-06
        o = num / den
        return (lambda x, *d: x.transpose(*d))(o, 0, 2, 1, 3).reshape(B, S, D) @ wo

    def _B_ref(x, w_in, w_sp, b_sp, w_out):
        B, S, D = x.shape
        F = w_in.shape[-1]
        Fh = F // 2
        z = _gelu(jnp.einsum('bsd,df->bsf', x, w_in))
        z1 = z[..., :Fh].copy()
        z2 = _layernorm(z[..., Fh:], axis=-1)
        g = jnp.einsum('ts,bsf->btf', w_sp, z2) + b_sp[None, :, None]
        return jnp.einsum('bsf,fd->bsd', z1 * g, w_out)
    x = A_x
    x = x + _A_ref(_layernorm(x, axis=-1), A_wqkv, A_w_phi, A_wo)
    x = x + _B_ref(_layernorm(x, axis=-1), B_w_in, B_w_sp, B_b_sp, B_w_out)
    x = x + _A_ref(_layernorm(x, axis=-1), A_wqkv, A_w_phi, A_wo)
    x = x + _B_ref(_layernorm(x, axis=-1), B_w_in, B_w_sp, B_b_sp, B_w_out)
    return x

def setup_inputs():
    _inp = _fwd_setup_inputs()
    _gk = jax.random.fold_in(jax.random.key(int.from_bytes(__import__("os").urandom(4), "little")), 2 ** 31 - 1)
    _shapes = [[1, 2048, 640]]
    _dtypes = ['bfloat16']
    _gks = jax.random.split(_gk, len(_shapes))
    _gs = [jax.random.normal(k, s, dtype=jnp.dtype(d)) * 0.05 for k, s, d in zip(_gks, _shapes, _dtypes)]
    _inp['grad_out'] = _gs[0]
    return _inp

def reference(A_x, A_wqkv, A_w_phi, A_wo, B_w_in, B_w_sp, B_b_sp, B_w_out, B_x, grad_out):
    _const = dict(B_x=B_x)

    def _f(*_d):
        return _fwd_reference(**{'A_x': _d[0], 'A_wqkv': _d[1], 'A_w_phi': _d[2], 'A_wo': _d[3], 'B_w_in': _d[4], 'B_w_sp': _d[5], 'B_b_sp': _d[6], 'B_w_out': _d[7], **_const})
    _out, _vjp = jax.vjp(_f, A_x, A_wqkv, A_w_phi, A_wo, B_w_in, B_w_sp, B_b_sp, B_w_out)
    _grads = _vjp(grad_out)
    _out0 = jnp.asarray(_out)
    return (_out0, *[jnp.asarray(_g) for _g in _grads])
```

```python
import functools

import jax
import jax.numpy as jnp
from jax import lax
import jax.experimental.pallas as pl
import jax.experimental.pallas.tpu as pltpu

F32 = jnp.float32
BF16 = jnp.bfloat16
S, D, H, DH, FF, FH = 2048, 640, 32, 20, 1536, 768
G = 4
GR = 8 * DH
GE = GR + 16
T = 256
NT_ = S // T
EPS = 1e-5
K0 = 0.7978845608028654
K1 = 0.044715


def _nn(a, b):
    return lax.dot_general(a, b, (((1,), (0,)), ((), ())), preferred_element_type=F32)


def _nt(a, b):
    return lax.dot_general(a, b, (((1,), (1,)), ((), ())), preferred_element_type=F32)


def _ln_rows(x):
    mu = jnp.mean(x, axis=0, keepdims=True)
    xc = x - mu
    var = jnp.mean(xc * xc, axis=0, keepdims=True)
    rstd = lax.rsqrt(var + EPS)
    return xc * rstd, rstd


def _ln_rows_bwd(dh, h, rstd):
    m1 = jnp.mean(dh, axis=0, keepdims=True)
    m2 = jnp.mean(dh * h, axis=0, keepdims=True)
    return (dh - m1 - h * m2) * rstd


def _softmax_pm(p):
    p3 = p.reshape(DH, 8, p.shape[-1])
    ep = jnp.exp(p3 - jnp.max(p3, axis=0, keepdims=True))
    en = jnp.exp(jnp.min(p3, axis=0, keepdims=True) - p3)
    ep = ep * (1.0 / jnp.sum(ep, axis=0, keepdims=True))
    en = en * (1.0 / jnp.sum(en, axis=0, keepdims=True))
    return ep.reshape(p.shape), en.reshape(p.shape)


def _softmax_pm_bwd(phi, dphi):
    t = phi.shape[-1]
    a = phi.reshape(2, DH, 8, t)
    da = dphi.reshape(2, DH, 8, t)
    r = a * (da - jnp.sum(a * da, axis=1, keepdims=True))
    return (r[0] - r[1]).reshape(GR, t)


def _perm_maps(shape, cdim):
    c = lax.broadcasted_iota(jnp.int32, shape, cdim)
    r = lax.broadcasted_iota(jnp.int32, shape, 1 - cdim)
    hg = ((c >= GR).astype(jnp.int32) + (c >= 2 * GR).astype(jnp.int32)
          + (c >= 3 * GR).astype(jnp.int32))
    cf = lax.shift_right_logical(c - hg * GR, 3)
    ch = hg * 8 + (c & 7)
    rh = lax.shift_right_logical(r * 3277, 16)
    rd = r - rh * DH
    return ch == rh, (ch == rh) & (cf == rd)


def _fsel(shape, cdim):
    c = lax.broadcasted_iota(jnp.int32, shape, cdim)
    f = lax.broadcasted_iota(jnp.int32, shape, 1 - cdim)
    hg = ((c >= GR).astype(jnp.int32) + (c >= 2 * GR).astype(jnp.int32)
          + (c >= 3 * GR).astype(jnp.int32))
    cf = lax.shift_right_logical(c - hg * GR, 3)
    return jnp.where(cf == f, 1.0, 0.0).astype(BF16)


def _win(g):
    return slice(128 * g, 128 * g + 256)


def _grp(g):
    return slice(GR * g, GR * (g + 1))


def _bd_rows(bd, fn):
    return jnp.concatenate([fn(bd[_grp(g), _win(g)], _win(g)) for g in range(G)], axis=0)


def _bd_cols(a, bd):
    outs = []
    for n in range(D // 128):
        k = slice(max(n - 1, 0) * 128, min(n + 2, D // 128) * 128)
        outs.append(_nn(a[:, k], bd[k, n * 128:(n + 1) * 128]))
    return jnp.concatenate(outs, axis=1)


def _loop(n, body, name):
    with jax.named_scope(name):
        lax.fori_loop(0, n, lambda j, _: body(j), None)


def _skew(s1, s2, name):
    with jax.named_scope(name):
        def body(j, cy):
            nxt = s1(j + 1)
            s2(j, cy)
            return nxt
        s2(NT_ - 1, lax.fori_loop(0, NT_ - 1, body, s1(0)))


def _cols(j):
    if isinstance(j, int):
        return pl.ds(j * T, T)
    return pl.ds(pl.multiple_of(j * T, T), T)


def _kernel(x_hbm, wqkv_hbm, wphi_hbm, wo_hbm, win_hbm, wsp_hbm, bsp_hbm, wout_hbm, go_hbm,
            out_hbm, gx_hbm, dwqkv_hbm, dwphi_hbm, dwo_hbm, dwin_hbm, dwsp_hbm, dbsp_hbm, dwout_hbm,
            nat_a, nat_b, xT, WpT, Wp, woT, wop, winT, win, woutT, wout, wsp, bsp, BDt,
            hA, rsA, phiq, phik, vext, oA, invA, kvT, kvTb, kvb,
            h1, rs1, gp1, z11, g1, rz1, z2, dgN2, dwin_acc, dwout_acc, db_acc, sems):
    def cp(src, dst, k):
        return pltpu.make_async_copy(src, dst, sems.at[k])

    c_x = cp(x_hbm, nat_a, 0)
    c_win = cp(win_hbm, win, 1)
    c_wout = cp(wout_hbm, wout, 2)
    c_wsp = cp(wsp_hbm, wsp, 3)
    c_bsp = cp(bsp_hbm, bsp, 4)
    c_go = cp(go_hbm, nat_b, 5)

    def prep(wraw, wphi, wo_raw):
        c_phi = cp(wphi_hbm, wphi, 6)
        c_w = cp(wqkv_hbm, wraw, 7)
        c_wo = cp(wo_hbm, wo_raw, 8)
        c_phi.start(); c_w.start(); c_x.start(); c_wo.start()
        same, pm = _perm_maps((D, D), 0)
        pmT = jnp.where(pm, 1.0, 0.0).astype(BF16)
        c_phi.wait()
        bdt = jnp.where(same, _nt(_fsel((D, DH), 0), wphi[...]), 0.0).astype(BF16)
        BDt[...] = bdt
        c_w.wait()
        WpT[0:D, :] = _bd_rows(bdt, lambda b, w: _nt(b, wraw[:, 0 * D + w.start:0 * D + w.stop])).astype(BF16)
        WpT[D:2 * D, :] = _bd_rows(bdt, lambda b, w: _nt(b, wraw[:, 1 * D + w.start:1 * D + w.stop])).astype(BF16)
        WpT[2 * D:3 * D, :] = _bd_rows(pmT, lambda b, w: _nt(b, wraw[:, 2 * D + w.start:2 * D + w.stop])).astype(BF16)
        c_wo.wait()
        wp_ = _bd_rows(pmT, lambda b, w: _nn(b, wo_raw[w, :]))
        wop[...] = wp_.astype(BF16)
        woT[...] = wp_.T.astype(BF16)

    pl.run_scoped(prep, pltpu.VMEM((D, 3 * D), BF16), pltpu.VMEM((D, DH), BF16),
                  pltpu.VMEM((D, D), BF16))

    ext_rows = lax.broadcasted_iota(jnp.int32, (16, S), 0)
    ext_c = jnp.where(ext_rows < 8, 1.0, 0.0).astype(BF16)
    for l in range(2):
        for g in range(G):
            vext[l, g, GR:GE, :] = ext_c

    km_r = lax.broadcasted_iota(jnp.int32, (GE, 2 * GR), 0)
    km_c = lax.broadcasted_iota(jnp.int32, (GE, 2 * GR), 1)
    kmask = (km_r & 7) == (km_c & 7)

    def zero_kv():
        kvT[...] = jnp.zeros(kvT.shape, F32)

    def finish_kv(l):
        for g in range(G):
            k = jnp.where(kmask, kvT[g], 0.0)
            kvTb[l, g] = k.astype(BF16)
            kvb[l, g] = k.T.astype(BF16)

    def ln_store(x, c, h_ref, rs_ref):
        xT[:, c] = x
        h, rstd = _ln_rows(x)
        hb = h.astype(BF16)
        h_ref[:, c] = hb
        rs_ref[:, c] = rstd
        return hb

    def a_fwd0(j):
        c = _cols(j)
        return ln_store(nat_a[c, :].astype(F32).T, c, hA.at[0], rsA.at[0])

    def a_fwd1(l, first):
        def body(j, hb):
            c = _cols(j)
            pk = _nn(WpT[D:2 * D, :], hb)
            v = _nn(WpT[2 * D:3 * D, :], hb)
            pq = _nn(WpT[0:D, :], hb)
            for g in range(G):
                ep, en = _softmax_pm(pk[g * GR:(g + 1) * GR])
                phik[l, g, 0:GR, c] = ep.astype(BF16)
                phik[l, g, GR:2 * GR, c] = en.astype(BF16)
                vext[l, g, 0:GR, c] = v[g * GR:(g + 1) * GR].astype(BF16)
                kvT[g] += _nt(vext[l, g, :, c], phik[l, g, :, c])
            for g in range(G):
                ep, en = _softmax_pm(pq[g * GR:(g + 1) * GR])
                phiq[l, g, 0:GR, c] = ep.astype(BF16)
                phiq[l, g, GR:2 * GR, c] = en.astype(BF16)
        return body

    def a_fwd2(l, hB, rsB):
        def body(j):
            c = _cols(j)
            for g in range(G):
                ne = _nn(kvTb[l, g], phiq[l, g, :, c])
                inv = 1.0 / (ne[GR:GR + 8] + 1e-6)
                invA[l, g, :, c] = inv
                o = ne[0:GR].reshape(DH, 8, T) * inv[None]
                oA[l, g * GR:(g + 1) * GR, c] = o.reshape(GR, T).astype(BF16)
            return ln_store(xT[:, c] + _nn(woT[...], oA[l, :, c]), c, hB, rsB)
        return body

    def b_fwd1(l, hB, rsB, gp, z1, rz):
        def body(j, hb):
            c = _cols(j)
            for half in (1, 0):
                u = _nn(winT[half * FH:(half + 1) * FH, :], hb)
                u2 = u * u
                t = jnp.tanh(u * (K0 + (K0 * K1) * u2))
                cdf = 0.5 + 0.5 * t
                z = u * cdf
                gpv = cdf + (0.5 * u) * (1.0 - t * t) * (K0 + (3 * K0 * K1) * u2)
                gp[half * FH:(half + 1) * FH, c] = gpv.astype(BF16)
                if half == 0:
                    z1[:, c] = z.astype(BF16)
                else:
                    zn, r2 = _ln_rows(z)
                    z2[l, :, c] = zn.astype(BF16)
                    rz[:, c] = r2
        return body

    def b_fwd2(l, z1, gb, last):
        def body(j):
            c = _cols(j)
            gv = _nt(z2[l], wsp[c, :]) + bsp[:, c].astype(F32)
            gb[:, c] = gv.astype(BF16)
            m = (z1[:, c].astype(F32) * gv).astype(BF16)
            xn = xT[:, c] + _nn(woutT[...], m)
            if last:
                nat_a[c, :] = xn.T.astype(BF16)
                xT[:, c] = nat_b[c, :].astype(F32).T
            else:
                return ln_store(xn, c, hA.at[1], rsA.at[1])
        return body

    def b_bwd1(gp, z1, gb, dgN):
        def body(j):
            c = _cols(j)
            dy = xT[:, c].astype(BF16)
            dm = _nn(wout[...], dy)
            gv = gb[:, c].astype(F32)
            zv = z1[:, c].astype(F32)
            dwout_acc[...] += _nt((zv * gv).astype(BF16), dy)
            gp[0:FH, c] = (dm * gv * gp[0:FH, c].astype(F32)).astype(BF16)
            dg = dm * zv
            gb[:, c] = dg.astype(BF16)
            dgN[c, :] = dg.T.astype(BF16)
            db_acc[:, c] += jnp.sum(dg, axis=0, keepdims=True)
        _loop(NT_, body, "b_bwd1")

    def b_bwd2(l, hB, rsB, gp, gb, rz):
        def body(j):
            c = _cols(j)
            dz = _nn(gb[...], wsp[:, c])
            dz = _ln_rows_bwd(dz, z2[l, :, c].astype(F32), rz[:, c])
            return (dz * gp[FH:FF, c].astype(F32)).astype(BF16)

        def body2(j, du2):
            c = _cols(j)
            du = jnp.concatenate([gp[0:FH, c], du2], axis=0)
            hb = hB[:, c]
            dh = _nn(win[...], du)
            xT[:, c] += _ln_rows_bwd(dh, hb.astype(F32), rsB[:, c])
            dwin_acc[...] += _nt(hb, du)
        _skew(body, body2, "b_bwd2")

    zero_kv()
    c_x.wait()
    c_win.start(); c_wout.start(); c_bsp.start(); c_wsp.start(); c_go.start()
    _skew(a_fwd0, a_fwd1(0, True), "a_fwd1")
    finish_kv(0)
    for k in range(3):
        Wp[:, k * D:(k + 1) * D] = WpT[k * D:(k + 1) * D, :].astype(F32).T.astype(BF16)
    c_win.wait()
    winT[...] = win[...].astype(F32).T.astype(BF16)
    c_wout.wait()
    woutT[...] = wout[...].astype(F32).T.astype(BF16)
    _skew(a_fwd2(0, h1, rs1), b_fwd1(0, h1, rs1, gp1, z11, rz1), "a2b1")
    c_wsp.wait()
    c_bsp.wait()
    zero_kv()
    _skew(b_fwd2(0, z11, g1, False), a_fwd1(1, False), "b2a1")
    finish_kv(1)

    dwin_acc[...] = jnp.zeros(dwin_acc.shape, F32)
    dwout_acc[...] = jnp.zeros(dwout_acc.shape, F32)
    db_acc[...] = jnp.zeros(db_acc.shape, F32)
    c_out = cp(nat_a, out_hbm, 9)

    def layer_b2(h2, rs2, gp2, z12, g2, rz2):
        _skew(a_fwd2(1, h2, rs2), b_fwd1(1, h2, rs2, gp2, z12, rz2), "a2b1")
        c_go.wait()
        _loop(NT_, b_fwd2(1, z12, g2, True), "b_fwd2")
        c_out.start()
        b_bwd1(gp2, z12, g2, dgN2)
        b_bwd2(1, h2, rs2, gp2, g2, rz2)

    pl.run_scoped(layer_b2, pltpu.VMEM((D, S), BF16), pltpu.VMEM((1, S), F32),
                  pltpu.VMEM((FF, S), BF16), pltpu.VMEM((FH, S), BF16),
                  pltpu.VMEM((FH, S), BF16), pltpu.VMEM((1, S), F32))

    def tail(dWp_acc, dwo_acc, dgN1, wraw, dphi_st, db_st):
        def a_bwd1(l):
            kvT[...] = jnp.zeros(kvT.shape, F32)

            def body(j):
                c = _cols(j)
                dy = xT[:, c].astype(BF16)
                do = _nn(wop[...], dy)
                dwo_acc[...] += _nt(oA[l, :, c], dy)
                for g in range(G):
                    inv = invA[l, g, :, c]
                    dn = do[g * GR:(g + 1) * GR].reshape(DH, 8, T) * inv[None]
                    o = oA[l, g * GR:(g + 1) * GR, c].astype(F32).reshape(DH, 8, T)
                    dden = -jnp.sum(dn * o, axis=0)
                    ext = jnp.concatenate(
                        [dn.reshape(GR, T), dden, jnp.zeros((8, T), F32)], axis=0).astype(BF16)
                    ph = phiq[l, g, :, c]
                    kvT[g] += _nt(ext, ph)
                    dphi = _nn(kvb[l, g], ext)
                    phiq[l, g, 0:GR, c] = _softmax_pm_bwd(ph.astype(F32), dphi).astype(BF16)
            _loop(NT_, body, "a_bwd1")
            finish_kv(l)

        def a_bwd2(l, last):
            def body(j):
                c = _cols(j)
                dk, dv = [], []
                for g in range(G):
                    ph = phik[l, g, :, c]
                    dphi = _nn(kvb[l, g], vext[l, g, :, c])
                    dk.append(_softmax_pm_bwd(ph.astype(F32), dphi).astype(BF16))
                    dv.append(_nn(kvTb[l, g, 0:GR, :], ph).astype(BF16))
                return jnp.concatenate(dk + dv, axis=0)

            def body2(j, dkv):
                c = _cols(j)
                hb = hA[l, :, c]
                dp = jnp.concatenate([phiq[l, g, 0:GR, c] for g in range(G)] + [dkv], axis=0)
                dh = _nn(Wp[...], dp)
                dx = xT[:, c] + _ln_rows_bwd(dh, hb.astype(F32), rsA[l, :, c])
                if last:
                    nat_b[c, :] = dx.T.astype(BF16)
                else:
                    xT[:, c] = dx
                dWp_acc[...] += _nt(hb, dp)
            _skew(body, body2, "a_bwd2")

        c_w = cp(wqkv_hbm, wraw, 6)
        c_w.start()
        dWp_acc[...] = jnp.zeros(dWp_acc.shape, F32)
        dwo_acc[...] = jnp.zeros(dwo_acc.shape, F32)
        a_bwd1(1)
        a_bwd2(1, False)
        b_bwd1(gp1, z11, g1, dgN1)

        wout[...] = dwout_acc[...].astype(BF16)
        c_dwout = cp(wout, dwout_hbm, 10)
        c_dwout.start()
        db_st[...] = db_acc[...].astype(BF16)
        c_db = cp(db_st, dbsp_hbm, 11)
        c_db.start()

        b_bwd2(0, h1, rs1, gp1, g1, rz1)

        def sp_copy(i):
            return pltpu.make_async_copy(wsp.at[_cols(i), :], dwsp_hbm.at[_cols(i), :], sems.at[3])

        def sp_body(i):
            r = _cols(i)
            wsp[r, :] = (_nn(dgN1[r, :], z2[0]) + _nn(dgN2[r, :], z2[1])).astype(BF16)
            sp_copy(i).start()
        _loop(NT_, sp_body, "dwsp")
        win[...] = dwin_acc[...].astype(BF16)
        c_dwin = cp(win, dwin_hbm, 12)
        c_dwin.start()
        a_bwd1(0)
        same_rc, pm_rc = _perm_maps((D, D), 1)
        woT[...] = _bd_rows(jnp.where(pm_rc, 1.0, 0.0).astype(BF16),
                            lambda b, w: _nn(b, dwo_acc[w, :].astype(BF16))).astype(BF16)
        c_dwo = cp(woT, dwo_hbm, 13)
        c_dwo.start()
        a_bwd2(0, True)
        c_gx = cp(nat_b, gx_hbm, 7)
        c_gx.start()

        _, pm_cr = _perm_maps((D, D), 0)
        dq = dWp_acc[:, 0:D].astype(BF16)
        dk = dWp_acc[:, D:2 * D].astype(BF16)
        Wp[:, 0:D] = _bd_cols(dq, BDt).astype(BF16)
        Wp[:, D:2 * D] = _bd_cols(dk, BDt).astype(BF16)
        Wp[:, 2 * D:3 * D] = _bd_cols(dWp_acc[:, 2 * D:3 * D].astype(BF16),
                                 jnp.where(pm_cr, 1.0, 0.0).astype(BF16)).astype(BF16)
        c_dwqkv = cp(Wp, dwqkv_hbm, 8)
        c_dwqkv.start()
        c_w.wait()
        wqT = wraw[:, 0:D].astype(F32).T.astype(BF16)
        wkT = wraw[:, D:2 * D].astype(F32).T.astype(BF16)
        fsel = _fsel((D, DH), 0)
        for g in range(G):
            r, w = _grp(g), _win(g)
            m = _nn(wqT[r], dq[:, w]) + _nn(wkT[r], dk[:, w])
            dphi_st[r, :] = _nn(jnp.where(same_rc[r, w], m, 0.0).astype(BF16),
                                fsel[w]).astype(BF16)
        c_dphi = cp(dphi_st, dwphi_hbm, 4)
        c_dphi.start()
        c_out.wait()
        for i in range(NT_):
            sp_copy(i).wait()
        c_dwout.wait(); c_db.wait(); c_dwin.wait(); c_dwo.wait()
        c_gx.wait(); c_dwqkv.wait(); c_dphi.wait()

    pl.run_scoped(tail, pltpu.VMEM((D, 3 * D), F32), pltpu.VMEM((D, D), F32),
                  pltpu.VMEM((S, FH), BF16),
                  pltpu.VMEM((D, 3 * D), BF16),
                  pltpu.VMEM((D, DH), BF16), pltpu.VMEM((1, S), BF16))


@jax.jit
def pallas_interleave_layers__linear_kernel_hedgehog__mixer_gmlp__prompt_kernel(
    A_x: jax.Array,
    A_wqkv: jax.Array,
    A_w_phi: jax.Array,
    A_wo: jax.Array,
    B_x: jax.Array,
    B_w_in: jax.Array,
    B_w_sp: jax.Array,
    B_b_sp: jax.Array,
    B_w_out: jax.Array,
    grad_out: jax.Array,
):
    del B_x
    V = pltpu.VMEM
    scratch = [
        V((S, D), BF16), V((S, D), BF16), V((D, S), F32),
        V((3 * D, D), BF16), V((D, 3 * D), BF16),
        V((D, D), BF16), V((D, D), BF16),
        V((FF, D), BF16), V((D, FF), BF16),
        V((D, FH), BF16), V((FH, D), BF16),
        V((S, S), BF16), V((1, S), BF16), V((D, D), BF16),
        V((2, D, S), BF16), V((2, 1, S), F32),
        V((2, G, 2 * GR, S), BF16), V((2, G, 2 * GR, S), BF16),
        V((2, G, GE, S), BF16), V((2, D, S), BF16), V((2, G, 8, S), F32),
        V((G, GE, 2 * GR), F32), V((2, G, GE, 2 * GR), BF16), V((2, G, 2 * GR, GE), BF16),
        V((D, S), BF16), V((1, S), F32), V((FF, S), BF16), V((FH, S), BF16),
        V((FH, S), BF16), V((1, S), F32), V((2, FH, S), BF16), V((S, FH), BF16),
        V((D, FF), F32), V((FH, D), F32), V((1, S), F32),
        pltpu.SemaphoreType.DMA((14,)),
    ]
    sds = jax.ShapeDtypeStruct
    out_shape = (sds((S, D), BF16), sds((S, D), BF16), sds((D, 3 * D), BF16),
                 sds((D, DH), BF16), sds((D, D), BF16), sds((D, FF), BF16),
                 sds((S, S), BF16), sds((1, S), BF16), sds((FH, D), BF16))
    anyspec = pl.BlockSpec(memory_space=pl.ANY)
    outs = pl.pallas_call(
        _kernel,
        out_shape=out_shape,
        in_specs=[anyspec] * 9,
        out_specs=[anyspec] * 9,
        scratch_shapes=scratch,
        compiler_params=pltpu.CompilerParams(vmem_limit_bytes=127 * 1024 * 1024),
    )(A_x.reshape(S, D), A_wqkv, A_w_phi.reshape(D, DH), A_wo, B_w_in, B_w_sp,
      B_b_sp.reshape(1, S), B_w_out, grad_out.reshape(S, D))
    out, gx, dwqkv, dwphi, dwo, dwin, dwsp, dbsp, dwout = outs
    return (out.reshape(1, S, D), gx.reshape(1, S, D), dwqkv, dwphi.reshape(H, DH, DH),
            dwo, dwin, dwsp, dbsp.reshape(S), dwout)
```
